```python
import os as _os
_os.environ.setdefault("JAX_PLATFORMS", "cpu")
import jax
import jax.numpy as jnp

def _softmax(x, axis=-1):
    return jax.nn.softmax(x, axis=axis)
def _gelu(x):
    return jax.nn.gelu(x, approximate=True)
def _silu(x):
    return jax.nn.silu(x)
def _sigmoid(x):
    return jax.nn.sigmoid(x)
def _layernorm(x, axis=-1, eps=1e-5):
    m = jnp.mean(x, axis=axis, keepdims=True)
    v = jnp.var(x, axis=axis, keepdims=True)
    return (x - m) / jnp.sqrt(v + eps)
def _scatter_add(tgt, idx, src, axis=0):
    return tgt.at[idx].add(src)
def _segment_sum(src, seg, n):
    return jax.ops.segment_sum(src, seg, n)
class _Rng:
    def __init__(self, key):
        self._k = key
    def _next(self):
        self._k, sub = jax.random.split(self._k)
        return sub
    def normal(self, shape):
        return jax.random.normal(self._next(), shape, dtype=jnp.bfloat16)
    def randint(self, lo, hi, shape):
        return jax.random.randint(self._next(), shape, lo, hi, dtype=jnp.int32)
    def uniform(self, shape, lo=0.0, hi=1.0):
        return jax.random.uniform(self._next(), shape, jnp.bfloat16, lo, hi)
    def permutation(self, n):
        return jax.random.permutation(self._next(), n)


kernel_name = 'standalone__linear_kernel_hedgehog__prompt'

def setup_inputs():
    _rng = _Rng(jax.random.key(int.from_bytes(__import__("os").urandom(4), "little")))
    _w = (lambda a: (lambda t: t.astype(jnp.bfloat16) if jnp.issubdtype(t.dtype, jnp.floating) else t)(jnp.asarray(a)))
    B, S, D, H = 1, 2048, 1024, 32
    Dh = D // H
    return {
        "x": _w((lambda *s: _rng.normal(s) * 0.4)(B, S, D)),
        "wqkv": _w((lambda *s: _rng.normal(s) * 0.4)(D, 3 * D)),
        "w_phi": _w((lambda *s: _rng.normal(s) * 0.4)(H, Dh, Dh) * (Dh ** -0.5)),
        "wo": _w((lambda *s: _rng.normal(s) * 0.05)(D, D)),
    }

def reference(x, wqkv, w_phi, wo):
    B, S, D = x.shape
    H = 32; Dh = D // H
    qkv = (lambda x, *d: x.transpose(*d))((x @ wqkv).reshape(B, S, 3, H, Dh), 2, 0, 3, 1, 4)
    q, k, v = qkv[0], qkv[1], qkv[2]
    pq = jnp.einsum("bhsd,hdf->bhsf", q, w_phi)
    pk = jnp.einsum("bhsd,hdf->bhsf", k, w_phi)
    phi_q = jnp.concatenate([_softmax(pq, axis=-1), _softmax(-pq, axis=-1)], axis=-1)
    phi_k = jnp.concatenate([_softmax(pk, axis=-1), _softmax(-pk, axis=-1)], axis=-1)
    kv = jnp.einsum("bhsf,bhsd->bhfd", phi_k, v)
    z  = jnp.einsum("bhsf->bhf", phi_k)
    num = jnp.einsum("bhqf,bhfd->bhqd", phi_q, kv)
    den = jnp.einsum("bhqf,bhf->bhq", phi_q, z)[..., None] + 1e-6
    o = num / den
    return (lambda x, *d: x.transpose(*d))(o, 0, 2, 1, 3).reshape(B, S, D) @ wo
```

```python
import functools
import numpy as np
import jax, jax.numpy as jnp
from jax import lax
from jax.experimental import pallas as pl
from jax.experimental.pallas import tpu as pltpu

S, D, H, DH = 2048, 1024, 32, 32
LOG2E = 1.4426950408889634
NT_DIMS = (((1,), (1,)), ((), ()))
F32, BF16 = jnp.float32, jnp.bfloat16

def nt(a, b):
    return lax.dot_general(a, b, NT_DIMS, preferred_element_type=F32)
def nn(a, b):
    return jnp.dot(a, b, preferred_element_type=F32)
def allred(m, op):
    m = op(m, pltpu.roll(m, 4, 0))
    m = op(m, pltpu.roll(m, 2, 0))
    return m
def recip(x):
    r = pl.reciprocal(x, approx=True)
    return r * (2.0 - x * r)
def tree(vals, op):
    vals = list(vals)
    while len(vals) > 1:
        vals = [op(vals[i], vals[i + 1]) if i + 1 < len(vals) else vals[i] for i in range(0, len(vals), 2)]
    return vals[0]
def fmap_tile(p):
    pv = [p[8*j:8*j+8, :] for j in range(8)]
    mx = allred(tree(pv, jnp.maximum), jnp.maximum)
    mn = allred(tree(pv, jnp.minimum), jnp.minimum)
    ep = [jnp.exp2(v - mx) for v in pv]
    rp = recip(allred(tree(ep, jnp.add), jnp.add))
    php = [e * rp for e in ep]
    en = [jnp.exp2(mn - v) for v in pv]
    rn = recip(allred(tree(en, jnp.add), jnp.add))
    phn = [e * rn for e in en]
    return php, phn
def pack(vals):
    return jnp.concatenate(vals, axis=0).astype(BF16)

def build(T1=128, RB1=1, LAG1=1, T2=256, RB2=8, LAG2=1, OSPLIT=False, LP=False, KVJOIN=True,
          PRO=512, WKC=(2, 3, 3), OUT_CHUNKS=None, flags=None, SCOPES=False, XR=(1024,), LASTSPLIT=False,
          FOLDQ_AT=1024, PERTILE1=True):
    if OUT_CHUNKS is None:
        OUT_CHUNKS = [(0, 1024), (1024, 1536), (1536, 1792), (1792, 2048)]
    assert sum(WKC) == 8 and PRO % 256 == 0 and PRO % T1 == 0

    def kernel(x_hbm, w_hbm, wphi_hbm, wo_hbm, o_hbm,
               x_v, w_v, wphi_v, wo_v, o_v, wTq, wTkv, pk_buf, kv_acc, z_acc, kvT, zb, oT, sems):
        def W(name, *cs):
            if SCOPES:
                with jax.named_scope(name):
                    for c in cs: c.wait()
            else:
                for c in cs: c.wait()
        nsem = [0]
        def cp(src, dst):
            i = nsem[0]; nsem[0] += 1
            return pltpu.make_async_copy(src, dst, sems.at[i])
        def wcols(c0, c1):
            return cp(w_hbm.at[:, pl.ds(c0, c1 - c0)], w_v.at[:, pl.ds(c0, c1 - c0)])
        def xrows(r0, r1):
            return cp(x_hbm.at[pl.ds(r0, r1 - r0), :], x_v.at[pl.ds(r0, r1 - r0), :])
        c_wphi = cp(wphi_hbm, wphi_v)
        gb = [0]
        for w in WKC: gb.append(gb[-1] + w)
        c_wk = [wcols(D + gb[i]*128, D + gb[i+1]*128) for i in range(len(WKC))]
        c_x0 = xrows(0, 256)
        c_xp = xrows(256, PRO) if PRO > 256 else None
        c_wv = wcols(2 * D, 3 * D)
        xb = [PRO] + list(XR) + [S]
        c_x = [xrows(xb[i], xb[i+1]) for i in range(len(xb) - 1)]
        c_wq = wcols(0, D)
        c_wo = cp(wo_hbm, wo_v)
        c_o = [cp(o_v.at[pl.ds(a, b - a), :], o_hbm.at[pl.ds(a, b - a), :]) for a, b in OUT_CHUNKS]
        order = [c_wphi, c_wk[0], c_x0] + c_wk[1:] + ([c_xp] if c_xp else []) + [c_wv] + c_x + [c_wq, c_wo]
        for c in order:
            c.start()

        r = lax.broadcasted_iota(jnp.int32, (128, 32), 0)
        c = lax.broadcasted_iota(jnp.int32, (128, 32), 1)
        pf = jnp.where(((r & 63) >> 1) == c, 1.0, 0.0).astype(BF16)
        r2 = lax.broadcasted_iota(jnp.int32, (128, 128), 0)
        c2 = lax.broadcasted_iota(jnp.int32, (128, 128), 1)
        hmask = (2 * (r2 >> 6) + (r2 & 1)) == (c2 >> 5)

        W('wphi', c_wphi)
        bdts = []
        for g in range(8):
            w4 = wphi_v[4*g:4*g+4].reshape(128, 32)
            bdts.append(jnp.where(hmask, nt(pf, w4), 0.0).astype(BF16))
        R1 = RB1 * 128
        def kvrow(part, g):
            b, i = divmod(g, RB1)
            return (b * 2 * RB1 + (part - 1) * RB1 + i) * 128
        def fold(part, g0, g1):
            for g in range(g0, g1):
                cols = w_v[:, part*D + g*128: part*D + (g+1)*128]
                val = (nt(bdts[g], cols) * LOG2E).astype(BF16)
                if part == 0:
                    wTq[g*128:(g+1)*128, :] = val
                else:
                    wTkv[kvrow(1, g):kvrow(1, g)+128, :] = val
        def kpro(g0, g1, t0, t1):
            xt = x_v[t0:t1, :]
            if RB1 == 8:
                pk_buf[g0*128:g1*128, t0:t1] = nt(wTkv[kvrow(1, g0):kvrow(1, g0) + (g1-g0)*128, :], xt)
            else:
                for g in range(g0, g1):
                    pk_buf[g*128:(g+1)*128, t0:t1] = nt(wTkv[kvrow(1, g):kvrow(1, g)+128, :], xt)
        for i in range(len(WKC)):
            if i == 0:
                W('wk0', c_wk[0], c_x0)
            else:
                W(f'wk{i}', c_wk[i])
            fold(1, gb[i], gb[i+1])
            kpro(gb[i], gb[i+1], 0, 256)
        if c_xp is not None:
            W('wxp', c_xp)
            kpro(0, 8, 256, PRO)
        W('wv', c_wv)
        for g in range(8):
            wTkv[kvrow(2, g):kvrow(2, g)+128, :] = w_v[:, 2*D + g*128: 2*D + (g+1)*128].T

        NJ1 = T1 // 128
        def kproj(n, b):
            xt = x_v[n*T1:(n+1)*T1, :]
            if n * T1 < PRO:
                pv = nt(wTkv[b*2*R1 + R1:(b+1)*2*R1, :], xt)
                pk = pk_buf[b*R1:(b+1)*R1, n*T1:(n+1)*T1]
            elif KVJOIN:
                res = nt(wTkv[b*2*R1:(b+1)*2*R1, :], xt)
                pk, pv = res[0:R1], res[R1:2*R1]
            else:
                pv = nt(wTkv[b*2*R1 + R1:(b+1)*2*R1, :], xt)
                pk = nt(wTkv[b*2*R1:b*2*R1 + R1, :], xt)
            return pv.astype(BF16), pk
        def kpost(n, b, vT, pk):
            for mm in range(2 * RB1):
                m = 2 * RB1 * b + mm
                lhs = vT[mm*64:(mm+1)*64, :]
                kv = None; zp = None; zn = None
                phis = []
                for j in range(NJ1):
                    php, phn = fmap_tile(pk[mm*64:(mm+1)*64, j*128:(j+1)*128])
                    zp = php if zp is None else [a + b_ for a, b_ in zip(zp, php)]
                    zn = phn if zn is None else [a + b_ for a, b_ in zip(zn, phn)]
                    phi = pack(php + phn)
                    if PERTILE1:
                        t = nt(lhs[:, j*128:(j+1)*128], phi)
                        kv = t if kv is None else kv + t
                    else:
                        phis.append(phi)
                if not PERTILE1:
                    kv = nt(lhs, jnp.concatenate(phis, axis=1))
                zz = jnp.concatenate(zp + zn, axis=0)
                if n == 0:
                    kv_acc[m] = kv
                    z_acc[m] = zz
                else:
                    kv_acc[m] += kv
                    z_acc[m] += zz

        units = [(n, b) for n in range(S // T1) for b in range(8 // RB1)]
        pend = []
        for (n, b) in units:
            if b == 0 and n * T1 in xb[:-1]:
                i = xb.index(n * T1)
                if i == len(xb) - 2:
                    W(f'wx{i}', c_x[i], c_wq, c_wo)
                else:
                    W(f'wx{i}', c_x[i])
            if b == 0 and n * T1 == FOLDQ_AT:
                fold(0, 0, 8)
            pend.append((n, b) + kproj(n, b))
            if len(pend) > LAG1:
                kpost(*pend.pop(0))
        R2 = RB2 * 128
        NJ2 = T2 // 128
        NB2 = 8 // RB2
        NT2 = S // T2
        def qproj(n, b):
            return nt(wTq[b*R2:(b+1)*R2, :], x_v[n*T2:(n+1)*T2, :])
        qunits = [(n, b) for n in range(NT2) for b in range(NB2)]
        qpend = []
        first = True
        while pend:
            if first or T2 * RB2 <= T1 * RB1:
                qpend.append(qunits[0] + (qproj(*qunits.pop(0)),))
            first = False
            kpost(*pend.pop(0))
        while len(qpend) < LAG2:
            qpend.append(qunits[0] + (qproj(*qunits.pop(0)),))
        r3 = lax.broadcasted_iota(jnp.int32, (64, 128), 0)
        c3 = lax.broadcasted_iota(jnp.int32, (64, 128), 1)
        kmask = (r3 >> 5) == (c3 & 1)
        for m in range(16):
            kvT[m] = jnp.where(kmask, kv_acc[m], 0.0).astype(BF16)
            zb[m] = jnp.broadcast_to(jnp.sum(z_acc[m], axis=1, keepdims=True), (128, 128))
        par = lax.broadcasted_iota(jnp.int32, (8, 128), 0) & 1

        def qpost(n, b, pq):
            for mm in range(2 * RB2):
                m = 2 * RB2 * b + mm
                lhs = kvT[m]
                for j in range(NJ2):
                    php, phn = fmap_tile(pq[mm*64:(mm+1)*64, j*128:(j+1)*128])
                    phi = pack(php + phn)
                    nd = nn(lhs, phi)
                    prods = [php[i] * zb[m, 8*i:8*i+8, :] for i in range(8)] + \
                            [phn[i] * zb[m, 64+8*i:64+8*i+8, :] for i in range(8)]
                    den = allred(tree(prods, jnp.add), jnp.add)
                    rd = recip(den + 1e-6)
                    rr = pltpu.roll(rd, 1, 0)
                    rd0 = jnp.where(par == 0, rd, rr)
                    rd1 = jnp.where(par == 1, rd, rr)
                    for i in range(8):
                        oT[n % 2, m*64 + 8*i: m*64 + 8*i + 8, j*128:(j+1)*128] = nd[8*i:8*i+8] * (rd0 if i < 4 else rd1)
        def ofinish(r1):
            for k, (a, b_) in enumerate(OUT_CHUNKS):
                if b_ == r1:
                    c_o[k].start()
        o = None
        for n in range(NT2 + 1):
            if n > 0:
                o = oT[(n - 1) % 2].T.astype(BF16)
                if not OSPLIT:
                    if LASTSPLIT and n == NT2:
                        for h in range(NJ2):
                            o_v[(n-1)*T2 + h*128:(n-1)*T2 + (h+1)*128, :] = nn(o[h*128:(h+1)*128], wo_v[...]).astype(BF16)
                            ofinish((n-1)*T2 + (h+1)*128)
                    else:
                        o_v[(n-1)*T2:n*T2, :] = nn(o, wo_v[...]).astype(BF16)
            for b in range(NB2):
                if qunits:
                    qpend.append(qunits[0] + (qproj(*qunits.pop(0)),))
                if n > 0 and OSPLIT:
                    Wd = 1024 // NB2
                    o_v[(n-1)*T2:n*T2, b*Wd:(b+1)*Wd] = nn(o, wo_v[:, b*Wd:(b+1)*Wd]).astype(BF16)
                if n < NT2:
                    qpost(*qpend.pop(0))
            if n > 0 and not (LASTSPLIT and n == NT2 and not OSPLIT):
                ofinish(n * T2)
        W('wout', *c_o)

    @jax.jit
    def fn(x, wqkv, w_phi, wo):
        x2 = x.reshape(S, D)
        any_spec = pl.BlockSpec(memory_space=pl.ANY)
        fl = dict(flags or {})
        if LP:
            fl["XLA_TPU_FORCE_LP_LLO_SCHEDULER"] = True
        out = pl.pallas_call(
            kernel,
            out_shape=jax.ShapeDtypeStruct((S, D), BF16),
            in_specs=[any_spec] * 4,
            out_specs=any_spec,
            scratch_shapes=[
                pltpu.VMEM((S, D), BF16),
                pltpu.VMEM((D, 3*D), BF16),
                pltpu.VMEM((H, DH, DH), BF16),
                pltpu.VMEM((D, D), BF16),
                pltpu.VMEM((S, D), BF16),
                pltpu.VMEM((D, D), BF16),
                pltpu.VMEM((2*D, D), BF16),
                pltpu.VMEM((D, PRO), F32),
                pltpu.VMEM((16, 64, 128), F32),
                pltpu.VMEM((16, 128, 128), F32),
                pltpu.VMEM((16, 64, 128), BF16),
                pltpu.VMEM((16, 128, 128), F32),
                pltpu.VMEM((2, D, T2), F32),
                pltpu.SemaphoreType.DMA((24,)),
            ],
            compiler_params=pltpu.CompilerParams(vmem_limit_bytes=100 << 20, flags=fl or None),
        )(x2, wqkv, w_phi, wo)
        return out.reshape(1, S, D)
    return fn


pallas_standalone__linear_kernel_hedgehog__prompt_kernel = build(PRO=512)
```

```python
import jax
import jax.numpy as jnp
from jax import lax
from jax.experimental import pallas as pl
from jax.experimental.pallas import tpu as pltpu

S, D, H, DH = 2048, 1024, 32, 32
T = 256
PRO = 512
LOG2E = 1.4426950408889634
F32, BF16 = jnp.float32, jnp.bfloat16


def _nt(a, b):
    return lax.dot_general(a, b, (((1,), (1,)), ((), ())), preferred_element_type=F32)


def _nn(a, b):
    return jnp.dot(a, b, preferred_element_type=F32)


def _tree(vals, op):
    vals = list(vals)
    while len(vals) > 1:
        vals = [op(vals[i], vals[i + 1]) for i in range(0, len(vals), 2)]
    return vals[0]


def _same_head(m, op):
    m = op(m, pltpu.roll(m, 4, 0))
    return op(m, pltpu.roll(m, 2, 0))


def _recip(x):
    r = pl.reciprocal(x, approx=True)
    return r * (2.0 - x * r)


def _feature_map(p):
    pv = [p[8 * j:8 * j + 8, :] for j in range(8)]
    mx = _same_head(_tree(pv, jnp.maximum), jnp.maximum)
    mn = _same_head(_tree(pv, jnp.minimum), jnp.minimum)
    ep = [jnp.exp2(v - mx) for v in pv]
    rp = _recip(_same_head(_tree(ep, jnp.add), jnp.add))
    pos = [e * rp for e in ep]
    en = [jnp.exp2(mn - v) for v in pv]
    rn = _recip(_same_head(_tree(en, jnp.add), jnp.add))
    neg = [e * rn for e in en]
    return pos, neg


def _kernel(x_hbm, w_hbm, wphi_hbm, wo_hbm, o_hbm,
            x_v, w_v, wphi_v, wo_v, o_v, wTq, wTkv, phi_buf, kv_acc, z_acc, kvT, zb,
            oT0, oT1, sems):
    oTs = (oT0, oT1)

    copies = {}

    def dma(name, src, dst):
        copies[name] = pltpu.make_async_copy(src, dst, sems.at[len(copies)])

    def dma_w(name, c0, c1):
        dma(name, w_hbm.at[:, pl.ds(c0, c1 - c0)], w_v.at[pl.ds(0, D), pl.ds(c0, c1 - c0)])

    def dma_x(name, r0, r1):
        dma(name, x_hbm.at[pl.ds(r0, r1 - r0), :], x_v.at[pl.ds(r0, r1 - r0), :])

    def dma_p(name, h0, h1):
        dma(name, wphi_hbm.at[pl.ds(h0, h1 - h0)], wphi_v.at[pl.ds(h0, h1 - h0)])

    dma_p("p0", 0, 8)
    dma_w("k01", D, D + 128)
    dma_x("x0", 0, 128)
    dma_w("k12", D + 128, D + 256)
    dma_x("x1", 128, 256)
    dma_p("p1", 8, 32)
    dma_w("k24", D + 256, D + 512)
    dma_w("k46", D + 512, D + 768)
    dma_w("k68", D + 768, D + 1024)
    dma_x("x2", 256, 512)
    dma_w("wv", 2 * D, 3 * D)
    dma_x("x3", 512, 1024)
    dma_x("x4", 1024, 2048)
    dma_w("wq", 0, D)
    dma("wo", wo_hbm, wo_v.at[pl.ds(0, D), :])
    inputs = list(copies)
    out_rows = ((0, 1024), (1024, 1536), (1536, 1792), (1792, 1920))
    for a, b in out_rows:
        dma(("o", b), o_v.at[pl.ds(a, b - a), :], o_hbm.at[pl.ds(a, b - a), :])
    for c in range(4):
        dma(("olast", c), o_v.at[pl.ds(S - 128, 128), pl.ds(c * 256, 256)],
            o_hbm.at[pl.ds(S - 128, 128), pl.ds(c * 256, 256)])
    for name in inputs:
        copies[name].start()

    hist = []

    def wait(*names, lag=2):
        if len(hist) >= lag:
            v = hist[-lag]
            if any(n[0] == "x" for n in names):
                x_v[S:S + 16, 0:128] = v
            if any(n[0] == "k" or n in ("wv", "wq") for n in names):
                w_v[D:D + 16, 0:128] = v
            if "wo" in names:
                wo_v[D:D + 16, 0:128] = v
            if any(n[0] == "p" for n in names):
                wphi_v[H, 0:16, :] = v[:, 0:DH]
        for n in names:
            copies[n].wait()

    r = lax.broadcasted_iota(jnp.int32, (128, DH), 0)
    c = lax.broadcasted_iota(jnp.int32, (128, DH), 1)
    pick_feature = jnp.where(((r & 63) >> 1) == c, 1.0, 0.0).astype(BF16)
    r2 = lax.broadcasted_iota(jnp.int32, (128, 128), 0)
    c2 = lax.broadcasted_iota(jnp.int32, (128, 128), 1)
    head_match = (2 * (r2 >> 6) + (r2 & 1)) == (c2 >> 5)
    bdt = {}

    def make_bdt(g0, g1):
        for g in range(g0, g1):
            w4 = wphi_v[4 * g:4 * g + 4].reshape(128, DH)
            bdt[g] = jnp.where(head_match, _nt(pick_feature, w4), 0.0).astype(BF16)
            hist.append(bdt[g][0:16, :])

    def fold(dst, row0, col0, g0, g1):
        for g in range(g0, g1):
            cols = w_v[0:D, col0 + g * 128:col0 + (g + 1) * 128]
            val = (_nt(bdt[g], cols) * LOG2E).astype(BF16)
            dst[row0 + g * 128:row0 + (g + 1) * 128, :] = val
            hist.append(val[0:16, 0:128])

    pk_pro = {}
    z_started = []

    def k_proj(g0, g1, t0, t1):
        xt = x_v[t0:t1, :]
        for g in range(g0, g1):
            res = _nt(wTkv[g * 128:(g + 1) * 128, :], xt)
            hist.append(res[0:16, 0:128].astype(BF16))
            for j in range((t1 - t0) // 128):
                pk_pro[g, t0 // 128 + j] = res[:, j * 128:(j + 1) * 128]

    def k_feat(g0, g1, t0, t1):
        for g in range(g0, g1):
            for mm in range(2):
                m = 2 * g + mm
                zz = None
                for j in range(t0 // 128, t1 // 128):
                    pos, neg = _feature_map(pk_pro[g, j][mm * 64:(mm + 1) * 64, :])
                    phi = jnp.concatenate(pos + neg, axis=0)
                    phi_buf[m, :, j * 128:(j + 1) * 128] = phi.astype(BF16)
                    zz = phi if zz is None else zz + phi
                if m in z_started:
                    z_acc[m] += zz
                else:
                    z_started.append(m)
                    z_acc[m] = zz

    def fold_k(g0, g1):
        fold(wTkv, 0, D, g0, g1)

    wait("p0")
    make_bdt(0, 2)
    wait("k01", "x0", lag=1)
    fold_k(0, 1)
    k_proj(0, 1, 0, 128)
    wait("k12", "x1")
    fold_k(1, 2)
    wait("p1")
    make_bdt(2, 8)
    k_proj(1, 2, 0, 256)
    k_proj(0, 1, 128, 256)
    wait("k24")
    fold_k(2, 4)
    k_proj(2, 4, 0, 256)
    k_feat(0, 2, 0, 256)
    wait("k46")
    fold_k(4, 6)
    k_proj(4, 6, 0, 256)
    k_feat(2, 4, 0, 256)
    wait("k68")
    fold_k(6, 8)
    k_proj(6, 8, 0, 256)
    k_feat(4, 6, 0, 256)
    wait("x2")
    k_proj(0, 8, 256, 512)
    k_feat(6, 8, 0, 256)
    k_feat(0, 4, 256, 512)
    wait("wv")
    for g in range(8):
        wTkv[D + g * 128:D + (g + 1) * 128, :] = w_v[0:D, 2 * D + g * 128:2 * D + (g + 1) * 128].T

    def v_proj(g):
        res = _nt(wTkv[D + g * 128:D + (g + 1) * 128, :], x_v[0:PRO, :]).astype(BF16)
        hist.append(res[0:16, 0:128])
        return res

    def kv_first(g, vT):
        for mm in range(2):
            kv_acc[2 * g + mm] = _nt(vT[mm * 64:(mm + 1) * 64, :], phi_buf[2 * g + mm])

    prev = None
    for g in range(8):
        cur = (g, v_proj(g))
        if g < 4:
            k_feat(4 + g, 5 + g, 256, 512)
        if prev is not None:
            kv_first(*prev)
        prev = cur

    def kv_proj(n):
        res = _nt(wTkv[...], x_v[n * T:(n + 1) * T, :])
        hist.append(res[0:16, 0:128].astype(BF16))
        return res[D:2 * D].astype(BF16), res[0:D]

    def kv_update(vT, pk):
        for m in range(16):
            lhs = vT[m * 64:(m + 1) * 64, :]
            kv = zz = None
            for j in range(T // 128):
                pos, neg = _feature_map(pk[m * 64:(m + 1) * 64, j * 128:(j + 1) * 128])
                phi = pos + neg
                zz = phi if zz is None else [a + b for a, b in zip(zz, phi)]
                t = _nt(lhs[:, j * 128:(j + 1) * 128], jnp.concatenate(phi, axis=0).astype(BF16))
                kv = t if kv is None else kv + t
            kv_acc[m] += kv
            z_acc[m] += jnp.concatenate(zz, axis=0)

    pending = None
    for n in range(PRO // T, S // T):
        if n * T == 512:
            wait("x3")
        if n * T == 1024:
            wait("x4", "wq", "wo")
            fold(wTq, 0, 0, 0, 8)
        cur = kv_proj(n)
        if pending is None:
            kv_first(*prev)
        else:
            kv_update(*pending)
        pending = cur

    def q_proj(n):
        return _nt(wTq[...], x_v[n * T:(n + 1) * T, :])

    pq = q_proj(0)
    kv_update(*pending)

    r3 = lax.broadcasted_iota(jnp.int32, (64, 128), 0)
    c3 = lax.broadcasted_iota(jnp.int32, (64, 128), 1)
    own_head = (r3 >> 5) == (c3 & 1)
    for m in range(16):
        kvT[m] = jnp.where(own_head, kv_acc[m], 0.0).astype(BF16)
        zb[m] = jnp.broadcast_to(jnp.sum(z_acc[m], axis=1, keepdims=True), (128, 128))
    parity = lax.broadcasted_iota(jnp.int32, (8, 128), 0) & 1

    def attend(n, pq):
        oT = oTs[n % 2]
        for m in range(16):
            lhs = kvT[m]
            for j in range(T // 128):
                pos, neg = _feature_map(pq[m * 64:(m + 1) * 64, j * 128:(j + 1) * 128])
                phi = pos + neg
                num = _nn(lhs, jnp.concatenate(phi, axis=0).astype(BF16))
                den = _tree([f * zb[m, 8 * i:8 * i + 8, :] for i, f in enumerate(phi)], jnp.add)
                rd = _recip(_same_head(den, jnp.add) + 1e-6)
                rr = pltpu.roll(rd, 1, 0)
                rds = (jnp.where(parity == 0, rd, rr), jnp.where(parity == 1, rd, rr))
                for i in range(8):
                    oT[m * 64 + 8 * i:m * 64 + 8 * i + 8, j * 128:(j + 1) * 128] = (
                        num[8 * i:8 * i + 8] * rds[i // 4])

    NT = S // T
    for n in range(NT):
        if n > 0:
            o = oTs[(n - 1) % 2][...].T.astype(BF16)
            o_v[(n - 1) * T:n * T, :] = _nn(o, wo_v[0:D, :]).astype(BF16)
        pq_next = q_proj(n + 1) if n + 1 < NT else None
        attend(n, pq)
        pq = pq_next
        if ("o", n * T) in copies:
            copies["o", n * T].start()
    o = oTs[(NT - 1) % 2][...].T.astype(BF16)
    o_v[S - 256:S - 128, :] = _nn(o[0:128], wo_v[0:D, :]).astype(BF16)
    copies["o", S - 128].start()
    for c in range(4):
        o_v[S - 128:S, c * 256:(c + 1) * 256] = _nn(
            o[128:256], wo_v[0:D, c * 256:(c + 1) * 256]).astype(BF16)
        copies["olast", c].start()
    for name in copies:
        if name not in inputs:
            copies[name].wait()


@jax.jit
def pallas_standalone__linear_kernel_hedgehog__prompt_kernel(
    x: jax.Array,
    wqkv: jax.Array,
    w_phi: jax.Array,
    wo: jax.Array,
):
    B = x.shape[0]
    assert x.shape == (1, S, D) and wqkv.shape == (D, 3 * D)
    assert w_phi.shape == (H, DH, DH) and wo.shape == (D, D)
    hbm = pl.BlockSpec(memory_space=pl.ANY)
    out = pl.pallas_call(
        _kernel,
        out_shape=jax.ShapeDtypeStruct((S, D), x.dtype),
        in_specs=[hbm] * 4,
        out_specs=hbm,
        scratch_shapes=[
            pltpu.VMEM((S + 16, D), BF16),
            pltpu.VMEM((D + 16, 3 * D), BF16),
            pltpu.VMEM((H + 1, DH, DH), BF16),
            pltpu.VMEM((D + 16, D), BF16),
            pltpu.VMEM((S, D), BF16),
            pltpu.VMEM((D, D), BF16),
            pltpu.VMEM((2 * D, D), BF16),
            pltpu.VMEM((16, 128, PRO), BF16),
            pltpu.VMEM((16, 64, 128), F32),
            pltpu.VMEM((16, 128, 128), F32),
            pltpu.VMEM((16, 64, 128), BF16),
            pltpu.VMEM((16, 128, 128), F32),
            pltpu.VMEM((D, T), F32),
            pltpu.VMEM((D, T), F32),
            pltpu.SemaphoreType.DMA((23,)),
        ],
        compiler_params=pltpu.CompilerParams(
            vmem_limit_bytes=100 << 20,
            disable_semaphore_checks=True,
            flags={"XLA_TPU_RESCHEDULE_DMA_DONES": True},
        ),
    )(x.reshape(S, D), wqkv, w_phi, wo)
    return out.reshape(B, S, D)
```
